```python
import os as _os
_os.environ.setdefault('JAX_PLATFORMS', 'cpu')
import jax
import jax.numpy as jnp

def _softmax(x, axis=-1):
    return jax.nn.softmax(x, axis=axis)

def _gelu(x):
    return jax.nn.gelu(x, approximate=True)

def _silu(x):
    return jax.nn.silu(x)

def _sigmoid(x):
    return jax.nn.sigmoid(x)

def _layernorm(x, axis=-1, eps=1e-05):
    m = jnp.mean(x, axis=axis, keepdims=True)
    v = jnp.var(x, axis=axis, keepdims=True)
    return (x - m) / jnp.sqrt(v + eps)

def _scatter_add(tgt, idx, src, axis=0):
    return tgt.at[idx].add(src)

def _segment_sum(src, seg, n):
    return jax.ops.segment_sum(src, seg, n)

class _Rng:

    def __init__(self, key):
        self._k = key

    def _next(self):
        self._k, sub = jax.random.split(self._k)
        return sub

    def normal(self, shape):
        return jax.random.normal(self._next(), shape, dtype=jnp.bfloat16)

    def randint(self, lo, hi, shape):
        return jax.random.randint(self._next(), shape, lo, hi, dtype=jnp.int32)

    def uniform(self, shape, lo=0.0, hi=1.0):
        return jax.random.uniform(self._next(), shape, jnp.bfloat16, lo, hi)

    def permutation(self, n):
        return jax.random.permutation(self._next(), n)
kernel_name = 'adaLN_cond__ssm_conv_h3__moe_arch_mod__prompt'

def setup_inputs():
    _rng = _Rng(jax.random.key(int.from_bytes(__import__("os").urandom(4), "little")))
    _w = lambda a: (lambda t: t.astype(jnp.bfloat16) if jnp.issubdtype(t.dtype, jnp.floating) else t)(jnp.asarray(a))

    def _A_setup():
        B, S, D = (1, 2048, 640)
        ks = 4
        return {'q': _w((lambda *s: _rng.normal(s) * 0.05)(B, S, D)), 'k': _w((lambda *s: _rng.normal(s) * 0.4)(B, S, D)), 'v': _w((lambda *s: _rng.normal(s) * 0.4)(B, S, D)), 'shift_k': _w((lambda *s: _rng.normal(s) * 0.4)(D, ks) * 0.5), 'ssm_k': _w((lambda *s: _rng.normal(s) * 0.4)(D, S) * (1.0 / S ** 0.5)), 'ssm_D': _w((lambda *s: _rng.normal(s) * 0.4)(D))}
    _A_in = _A_setup()

    def _B_setup():
        B, S, D, F, C = (1, 2048, 640, 1728, 2)
        return {'x': _w((lambda *s: _rng.normal(s) * 0.05)(B, S, D)), 'w_r': _w((lambda *s: _rng.normal(s) * 0.1)(D)), 'w_gate': _w((lambda *s: _rng.normal(s) * 0.1)(D, F)), 'w_up': _w((lambda *s: _rng.normal(s) * 0.1)(D, F)), 'w_down': _w((lambda *s: _rng.normal(s) * 0.1)(F, D))}
    _B_in = _B_setup()
    return {'A_q': _A_in['q'], 'A_k': _A_in['k'], 'A_v': _A_in['v'], 'A_shift_k': _A_in['shift_k'], 'A_ssm_k': _A_in['ssm_k'], 'A_ssm_D': _A_in['ssm_D'], 'B_x': _B_in['x'], 'B_w_r': _B_in['w_r'], 'B_w_gate': _B_in['w_gate'], 'B_w_up': _B_in['w_up'], 'B_w_down': _B_in['w_down'], 'c': _w((lambda *s: _rng.normal(s) * 0.2)(1, 640) * 8.0), 'w_mod': _w((lambda *s: _rng.normal(s) * 0.2)(640, 6 * 640) * 640 ** (-0.5) * 8.0)}

def reference(A_q, A_k, A_v, A_shift_k, A_ssm_k, A_ssm_D, B_x, B_w_r, B_w_gate, B_w_up, B_w_down, c, w_mod):

    def _A_ref(q, k, v, shift_k, ssm_k, ssm_D):
        B, S, D = q.shape
        ks = shift_k.shape[-1]
        k_pad = jnp.pad(k, ((0, 0), (ks - 1, 0), (0, 0)))
        k_shift = jnp.zeros_like(k)
        for t in range(ks):
            k_shift = k_shift + k_pad[:, t:t + S, :] * shift_k[:, ks - 1 - t][None, None, :]
        kv = k_shift * v
        L = 2 * S
        kv_pad = jnp.pad(kv, ((0, 0), (0, S), (0, 0)))
        kf_pad = jnp.pad(ssm_k, ((0, 0), (0, S)))
        kv_f = (lambda x, axes=(-2, -1): jnp.fft.rfft2(x.astype(jnp.float32), axes=axes))(kv_pad[:, None, :, :], axes=(1, 2))
        kf_f = (lambda x, axes=(-2, -1): jnp.fft.rfft2(x.astype(jnp.float32), axes=axes))(kf_pad[:, None, :], axes=(1, 2))
        kf_f = (lambda x, *d: x.transpose(*d))(kf_f, 1, 2, 0)
        y_f = kv_f * kf_f[None, :, :, :]
        y = (lambda x, s, axes=(-2, -1): jnp.fft.irfft2(x, s=s, axes=axes).astype(jnp.bfloat16))(y_f, (1, L), axes=(1, 2))[:, 0, :S, :]
        y = y + kv * ssm_D[None, None, :]
        return q * y

    def _B_ref(x, w_r, w_gate, w_up, w_down):
        B, S, D = x.shape
        C = 2
        r = x @ w_r
        idx = jnp.argsort(-r, axis=-1)[:, :C]
        idx_e = jnp.repeat(idx.reshape(B, C, 1), D, axis=2)
        x_sel = jnp.take_along_axis(x, idx_e, axis=1)
        g = _silu(x_sel @ w_gate)
        u = x_sel @ w_up
        y = g * u @ w_down
        r_sel = _sigmoid(jnp.take_along_axis(r, idx, axis=1))
        y = y * r_sel.reshape(B, C, 1)
        b_off = (jnp.arange(B) * S).reshape(B, 1)
        flat_idx = (idx + b_off).reshape(B * C)
        zero = (x * 0.0).reshape(B * S, D)
        upd = _scatter_add(zero, flat_idx, y.reshape(B * C, D), axis=0)
        return x + upd.reshape(B, S, D)
    x = A_q
    mod = (_silu(c) @ w_mod).reshape(c.shape[0], 6, 1, -1)
    sa, ca, ga, sb, cb, gb = (mod[:, 0].copy(), mod[:, 1].copy(), mod[:, 2].copy(), mod[:, 3].copy(), mod[:, 4].copy(), mod[:, 5].copy())
    h = _layernorm(x, axis=-1) * (1 + ca) + sa
    x = x + ga * _A_ref(h, A_k, A_v, A_shift_k, A_ssm_k, A_ssm_D)
    h = _layernorm(x, axis=-1) * (1 + cb) + sb
    x = x + gb * _B_ref(h, B_w_r, B_w_gate, B_w_up, B_w_down)
    return x
```

```python
import numpy as np
import jax
import jax.numpy as jnp
import jax.experimental.pallas as pl
import jax.experimental.pallas.tpu as pltpu

S, D, FF = 2048, 640, 1728
BL = 128
NB = S // BL
NG = D // 128
QB = 4
NQ = NB // QB
EPS = 1e-5
L2N = 2
f32, bf16, u32, i32 = jnp.float32, jnp.bfloat16, jnp.uint32, jnp.int32
NT = (((1,), (1,)), ((), ()))


def _pack_rows(m):
    b = np.asarray(m, np.float32).astype(jnp.bfloat16).view(np.uint16).astype(np.uint32)
    return b[0::2] | (b[1::2] << 16)


def _dft_consts():
    m = np.arange(BL)[:, None].astype(np.float64)
    n = np.arange(BL)[None, :].astype(np.float64)
    th = np.pi * (4.0 * m + 1.0) * n / (2.0 * BL)
    c, s = np.cos(th), np.sin(th)
    fu = np.concatenate([c, s - c, s + c], axis=0)
    fk = np.concatenate([c + s, c, -s], axis=0)
    gi = np.stack([c.T.reshape(BL, BL // 8, 8), s.T.reshape(BL, BL // 8, 8)], axis=2).reshape(BL, 2 * BL) / BL
    allm = np.concatenate([fu, fk, gi[:, :BL], gi[:, BL:]], axis=0)
    return _pack_rows(allm)


_CONSTS = _dft_consts()


def _kernel(q_hbm, k_hbm, v_hbm, shk_hbm, ssm_hbm, dv_hbm, wr_hbm, wg_hbm, wu_hbm, wd_hbm,
            c_hbm, wm_hbm, cst_hbm, out_hbm,
            qb, kb, vb, sb, wmb, wgb, wub, wdb, shk, dv, wr, cb, cst,
            kf, kvp, sp, ub0, ub1, kp0, kp1, ypk, ypk4, y1b, y2b, st1, x1b, st2, ob, par, rb, sems):
    ubs, kps = (ub0, ub1), (kp0, kp1)

    def cp(src, dst, s):
        return pltpu.make_async_copy(src, dst, sems.at[s])

    small = [cp(cst_hbm, cst, 0), cp(shk_hbm, shk, 0), cp(dv_hbm, dv, 0), cp(wr_hbm, wr, 0), cp(c_hbm, cb, 0)]
    RC = QB * BL

    def kv_chunk(slab, it):
        c0, w = ((0, 256), (256, 384))[slab]
        sem = 1 + slab * NQ + it
        rows = pl.ds(pl.multiple_of(it * RC, RC), RC)
        return [cp(k_hbm.at[0, rows, pl.ds(c0, w)], kb.at[rows, pl.ds(c0, w)], sem),
                cp(v_hbm.at[0, rows, pl.ds(c0, w)], vb.at[rows, pl.ds(c0, w)], sem)]

    def ssm_cp(g):
        return cp(ssm_hbm.at[pl.ds(g * 128, 128), :], sb.at[pl.ds(g * 128, 128), :], 9 + g)

    qc = cp(q_hbm.at[0], qb, 14)
    wmc = cp(wm_hbm, wmb, 15)
    wgc = cp(wg_hbm, wgb, 16)
    wuc = cp(wu_hbm, wub, 17)
    wdc = cp(wd_hbm, wdb, 18)
    order = small + [ssm_cp(0)]
    for it in range(NQ):
        order += kv_chunk(0, it)
    order += [ssm_cp(1), ssm_cp(2)]
    for it in range(NQ):
        order += kv_chunk(1, it)
    order += [ssm_cp(3), ssm_cp(4), qc, wmc, wgc, wuc, wdc]
    for c in order:
        c.start()
    for c in small:
        c.wait()

    shw = shk[...].astype(f32)
    for j in range(4):
        par[8 * j:8 * j + 8, :] = jnp.broadcast_to(shw[j:j + 1, :], (8, D))
    par[32:40, :] = jnp.broadcast_to(dv[...].astype(f32).reshape(1, D), (8, D))
    for g in range(NG):
        kf[g, 0:8, :] = jnp.zeros((8, 128), f32)

    def prep(g, it):
        lanes = slice(g * 128, (g + 1) * 128)
        for b in range(QB):
            r0 = pl.multiple_of(it * (QB * BL) + b * BL, BL)
            kblk = kb[pl.ds(r0, BL), lanes].astype(f32)
            kf[g, pl.ds(8 + r0, BL), :] = kblk
            acc = kblk.reshape(BL // 8, 8, 128) * par[0:8, lanes][None]
            for j in range(1, 4):
                acc = acc + kf[g, pl.ds(8 + r0 - j, BL), :].reshape(BL // 8, 8, 128) * par[8 * j:8 * j + 8, lanes][None]
            kv = (acc.reshape(BL, 128) * vb[pl.ds(r0, BL), lanes].astype(f32)).astype(bf16)
            kvp[g, it, :, b * 128:(b + 1) * 128] = pltpu.bitcast(kv, u32)
            sp[g, it, b * 64:(b + 1) * 64, :] = pltpu.bitcast(sb[lanes, pl.ds(r0, BL)], u32)

    def trans(g, it):
        slot = g % 2
        fu = pltpu.bitcast(cst[0:192, :], bf16)
        ubs[slot][it] = jnp.dot(fu, pltpu.bitcast(kvp[g, it], bf16), preferred_element_type=f32)
        fk = pltpu.bitcast(cst[192:384, :], bf16)
        kps[slot][it] = jax.lax.dot_general(fk, pltpu.bitcast(sp[g, it], bf16), NT, preferred_element_type=f32)

    def conv(g, rg):
        slot = g % 2
        lanes = slice(g * 128, (g + 1) * 128)
        r = pl.multiple_of(rg * 8, 8)
        dvec = par[32:40, lanes]

        def prod(comp, init):
            u = [ubs[slot][j // QB, pl.ds(comp * BL + r, 8), (j % QB) * 128:(j % QB + 1) * 128] for j in range(NB)]
            kk = [kps[slot][j // QB, pl.ds(comp * BL + r, 8), (j % QB) * 128:(j % QB + 1) * 128] for j in range(NB)]
            if comp < 2:
                kk[0] = kk[0] + dvec
            res = []
            for a in range(NB):
                acc = u[a] * kk[0]
                if init is not None:
                    acc = acc + init[a]
                for j in range(1, a + 1):
                    acc = acc + u[a - j] * kk[j]
                res.append(acc)
            return res

        s1_ = prod(0, None)
        zre = prod(2, s1_)
        zim = prod(1, s1_)
        for a in range(NB):
            yre = zre[a] if a == 0 else zre[a] + zim[a - 1]
            yim = zim[a] if a == 0 else zim[a] - zre[a - 1]
            yy = jnp.concatenate([yre, yim], axis=0).astype(bf16)
            if g < NG - 1:
                ypk[a, pl.ds(r, 8), lanes] = pltpu.bitcast(yy, u32)
            else:
                ypk4[a, pl.ds(r, 8), :] = pltpu.bitcast(yy, u32)

    def inv03(a):
        r0 = pl.multiple_of(a * BL, BL)
        g1 = pltpu.bitcast(cst[384:448, :], bf16)
        g2 = pltpu.bitcast(cst[448:512, :], bf16)
        y1b[pl.ds(r0, BL), 0:512] = jnp.dot(g1, pltpu.bitcast(ypk[a, 0:64, :], bf16), preferred_element_type=f32)
        y2b[pl.ds(r0, BL), 0:512] = jnp.dot(g2, pltpu.bitcast(ypk[a, 64:128, :], bf16), preferred_element_type=f32)

    def inv4(a0, n):
        g1 = pltpu.bitcast(cst[384:448, :], bf16)
        g2 = pltpu.bitcast(cst[448:512, :], bf16)
        w1 = jnp.concatenate([ypk4[a0 + b, 0:64, :] for b in range(n)], axis=1)
        w2 = jnp.concatenate([ypk4[a0 + b, 64:128, :] for b in range(n)], axis=1)
        o1 = jnp.dot(g1, pltpu.bitcast(w1, bf16), preferred_element_type=f32)
        o2 = jnp.dot(g2, pltpu.bitcast(w2, bf16), preferred_element_type=f32)
        for b in range(n):
            r0 = pl.multiple_of((a0 + b) * BL, BL)
            y1b[pl.ds(r0, BL), 512:640] = o1[:, b * 128:(b + 1) * 128]
            y2b[pl.ds(r0, BL), 512:640] = o2[:, b * 128:(b + 1) * 128]

    def stats(x, dst, r0):
        m = jnp.sum(x, axis=-1, keepdims=True) * (1.0 / D)
        ex2 = jnp.sum(x * x, axis=-1, keepdims=True) * (1.0 / D)
        rs = jax.lax.rsqrt(jnp.maximum(ex2 - m * m, 0.0) + EPS)
        dst[0, pl.ds(r0, BL), :] = jnp.broadcast_to(m, (BL, 128))
        dst[1, pl.ds(r0, BL), :] = jnp.broadcast_to(rs, (BL, 128))

    def ln1_stats(a):
        r0 = pl.multiple_of(a * BL, BL)
        stats(qb[pl.ds(r0, BL), :].astype(f32), st1, r0)

    def wait_kv(slab, it):
        for c in kv_chunk(slab, it):
            c.wait()

    ssm_cp(0).wait()
    for it in range(NQ):
        wait_kv(0, it)
        prep(0, it)
        if it > 0:
            trans(0, it - 1)
    ssm_cp(1).wait()
    prep(1, 0)
    trans(0, NQ - 1)

    def l1_body(g, it, last):
        for b in range(QB):
            conv(g, it * QB + b)
        if g + 1 < NG:
            trans(g + 1, it)
            if not last:
                prep(g + 1, it + 1)
            elif g + 2 < NG:
                prep(g + 2, 0)
        else:
            for b in range(QB):
                inv03(it * QB + b)
            for b in range(QB):
                ln1_stats(it * QB + b)

    for g in range(NG):
        if g == NG - 1:
            qc.wait()

            def l1(it, c, g=g):
                l1_body(g, it, False)
                return c
            jax.lax.fori_loop(0, NQ, l1, 0)
        else:
            def l1(it, c, g=g):
                if g == 1:
                    wait_kv(1, it + 1)
                l1_body(g, it, False)
                return c
            jax.lax.fori_loop(0, NQ - 1, l1, 0)
            if g == 0:
                wait_kv(1, 0)
            if g + 2 < NG:
                ssm_cp(g + 2).wait()
            l1_body(g, NQ - 1, True)

    wmc.wait()
    inv4(0, L2N)
    cv = cb[...].astype(f32)
    sc = (cv * jax.nn.sigmoid(cv)).astype(bf16)
    mod = jnp.dot(jnp.broadcast_to(sc, (8, D)), wmb[...], preferred_element_type=f32)
    sa, ca, ga, sb_, cb_, gb = [mod[:, j * D:(j + 1) * D] for j in range(6)]
    par[40:48, :] = ga * (1.0 + ca)
    par[48:56, :] = ga * sa
    par[56:64, :] = gb * (1.0 + cb_)
    par[64:72, :] = gb * sb_
    par[72:80, :] = 1.0 + cb_
    par[80:88, :] = sb_
    par[88:96, :] = gb
    wrv = jnp.broadcast_to(wr[...].astype(f32).reshape(1, D), (8, D))
    wp = (1.0 + cb_) * wrv
    wp_hi = wp.astype(bf16).astype(f32)
    row = jax.lax.broadcasted_iota(i32, (8, D), 0)
    par[96:104, :] = jnp.where(row == 0, wp_hi, jnp.where(row == 1, wp - wp_hi, 0.0))
    rconst = jnp.sum(sb_[0:1, :] * wrv[0:1, :], axis=-1, keepdims=True)

    def tile5(t):
        return jnp.concatenate([t] * NG, axis=1)

    def stage_a(i):
        r0 = pl.multiple_of(i * BL, BL)
        y = y1b[pl.ds(r0, BL), :] + y2b[pl.ds(r0, BL), :]
        x = qb[pl.ds(r0, BL), :].astype(f32)
        n1 = (x - tile5(st1[0, pl.ds(r0, BL), :])) * tile5(st1[1, pl.ds(r0, BL), :])
        t = n1.reshape(BL // 8, 8, D) * par[40:48, :][None] + par[48:56, :][None]
        x1 = x + t.reshape(BL, D) * y
        x1b[pl.ds(r0, BL), :] = x1
        stats(x1, st2, r0)

    def stage_b(i):
        r0 = pl.multiple_of(i * BL, BL)
        x1 = x1b[pl.ds(r0, BL), :]
        n2 = (x1 - tile5(st2[0, pl.ds(r0, BL), :])) * tile5(st2[1, pl.ds(r0, BL), :])
        t = n2.reshape(BL // 8, 8, D) * par[56:64, :][None] + par[64:72, :][None]
        ob[pl.ds(r0, BL), :] = (x1 + t.reshape(BL, D)).astype(bf16)
        rr = jax.lax.dot_general(par[96:104, :].astype(bf16), n2.astype(bf16), NT, preferred_element_type=f32)
        rb[pl.ds(i, 1), :] = rr[0:1, :] + rr[1:2, :]

    n2it = NB // L2N

    def l2_body(i, do_m, do_a, do_b):
        if do_b:
            for b in range(L2N):
                stage_b((i - 1) * L2N + b)
        if do_a:
            for b in range(L2N):
                stage_a(i * L2N + b)
        if do_m:
            inv4((i + 1) * L2N, L2N)

    l2_body(0, True, True, False)

    def l2(i, c):
        l2_body(i, True, True, True)
        return c
    jax.lax.fori_loop(1, n2it - 1, l2, 0)
    l2_body(n2it - 1, False, True, True)
    l2_body(n2it, False, False, True)

    r = rb[...] + rconst
    pos = jax.lax.broadcasted_iota(i32, (NB, BL), 0) * BL + jax.lax.broadcasted_iota(i32, (NB, BL), 1)
    posf = pos.astype(f32)
    m1 = jnp.max(jnp.max(r, axis=1, keepdims=True), axis=0, keepdims=True)
    p1 = jnp.min(jnp.min(jnp.where(r == m1, posf, float(S)), axis=1, keepdims=True), axis=0, keepdims=True)
    r2 = jnp.where(posf == p1, -jnp.inf, r)
    m2 = jnp.max(jnp.max(r2, axis=1, keepdims=True), axis=0, keepdims=True)
    p2 = jnp.min(jnp.min(jnp.where(r2 == m2, jnp.where(posf == p1, float(S), posf), float(S)), axis=1, keepdims=True), axis=0, keepdims=True)
    i1 = jnp.clip(p1[0, 0].astype(i32), 0, S - 1)
    i2 = jnp.clip(p2[0, 0].astype(i32), 0, S - 1)

    def out_cp(a):
        rows = pl.ds(pl.multiple_of(a * BL, BL), BL)
        return cp(ob.at[rows, :], out_hbm.at[0, rows, :], 19)

    a1 = i1 // BL
    a2 = i2 // BL
    for a in range(NB):
        @pl.when(jnp.logical_and(a1 != a, a2 != a))
        def _(a=a):
            out_cp(a).start()

    def sel_row(idx):
        x1 = x1b[pl.ds(idx, 1), :]
        n2 = (x1 - tile5(st2[0, pl.ds(idx, 1), :])) * tile5(st2[1, pl.ds(idx, 1), :])
        return x1, n2 * par[72:73, :] + par[80:81, :]
    xa, ha = sel_row(i1)
    xb, hb = sel_row(i2)
    row = jax.lax.broadcasted_iota(i32, (8, D), 0)
    hsel = jnp.where(row == 0, ha, jnp.where(row == 1, hb, 0.0))
    hs = hsel.astype(bf16)
    wgc.wait()
    gate = jax.lax.dot_general(hs, wgb[...], NT, preferred_element_type=f32)
    wuc.wait()
    up = jax.lax.dot_general(hs, wub[...], NT, preferred_element_type=f32)
    act = (gate * jax.nn.sigmoid(gate) * up).astype(bf16)
    wdc.wait()
    ymoe = jnp.dot(act, wdb[...], preferred_element_type=f32)
    gbv = par[88:89, :]
    oa = xa + gbv * (ha + ymoe[0:1, :] * jax.nn.sigmoid(m1))
    obb = xb + gbv * (hb + ymoe[1:2, :] * jax.nn.sigmoid(m2))
    row16 = jax.lax.broadcasted_iota(i32, (16, D), 0)
    for idx, val in ((i1, oa), (i2, obb)):
        base = pl.multiple_of((idx // 16) * 16, 16)
        blk = ob[pl.ds(base, 16), :].astype(f32)
        ob[pl.ds(base, 16), :] = jnp.where(row16 == idx - base, val, blk).astype(bf16)
    out_cp(a1).start()

    @pl.when(a2 != a1)
    def _():
        out_cp(a2).start()
    for a in range(NB):
        out_cp(a).wait()


@jax.jit
def pallas_adaLN_cond__ssm_conv_h3__moe_arch_mod__prompt_kernel(
    A_q, A_k, A_v, A_shift_k, A_ssm_k, A_ssm_D, B_x, B_w_r, B_w_gate, B_w_up, B_w_down, c, w_mod,
):
    del B_x
    anyspec = pl.BlockSpec(memory_space=pl.ANY)
    V = pltpu.VMEM
    scratch = [
        V((S, D), bf16), V((S, D), bf16), V((S, D), bf16), V((D, S), bf16),
        V((D, 6 * D), bf16), V((FF, D), bf16), V((FF, D), bf16), V((FF, D), bf16),
        V((4, D), bf16), V((D,), bf16), V((D,), bf16), V((1, D), bf16), V((512, 128), u32),
        V((NG, S + 8, 128), f32),
        V((NG, NQ, 64, QB * 128), u32),
        V((NG, NQ, QB * 64, 128), u32),
        V((NQ, 3 * BL, QB * 128), f32), V((NQ, 3 * BL, QB * 128), f32),
        V((NQ, 3 * BL, QB * 128), f32), V((NQ, 3 * BL, QB * 128), f32),
        V((NB, BL, 512), u32), V((NB, BL, 128), u32),
        V((S, D), f32), V((S, D), f32),
        V((2, S, 128), f32),
        V((S, D), f32),
        V((2, S, 128), f32),
        V((S, D), bf16),
        V((104, D), f32),
        V((NB, BL), f32),
        pltpu.SemaphoreType.DMA((20,)),
    ]
    return pl.pallas_call(
        _kernel,
        out_shape=jax.ShapeDtypeStruct((1, S, D), bf16),
        in_specs=[anyspec] * 13,
        out_specs=anyspec,
        scratch_shapes=scratch,
        compiler_params=pltpu.CompilerParams(vmem_limit_bytes=100 * 1024 * 1024,
                                             disable_bounds_checks=True, disable_semaphore_checks=True),
        name="ssm_moe",
    )(A_q, A_k, A_v, A_shift_k.T, A_ssm_k, A_ssm_D, B_w_r, B_w_gate.T, B_w_up.T, B_w_down, c, w_mod,
      jnp.asarray(_CONSTS))
```

```python
import numpy as np
import jax
import jax.numpy as jnp
import jax.experimental.pallas as pl
import jax.experimental.pallas.tpu as pltpu

S, D, FF = 2048, 640, 1728
BL = 128
NB = S // BL
NG = D // 128
QB = 4
NQ = NB // QB
RC = QB * BL
L2N = 2
NE = 4
SPLIT = (10, 16)
EPS = 1e-5
f32, bf16, u32, i32 = jnp.float32, jnp.bfloat16, jnp.uint32, jnp.int32
NT = (((1,), (1,)), ((), ()))
NN = (((1,), (0,)), ((), ()))

P_SH, P_D, P_A1, P_B1, P_A2, P_B2, P_C2, P_S2, P_G2, P_WR, P_END = 0, 32, 40, 48, 56, 64, 72, 80, 88, 96, 104
S_SMALL, S_KV, S_SSM, S_Q, S_WM, S_WG, S_WU, S_WD, S_OE, S_OL, S_END = 0, 1, 9, 14, 15, 16, 17, 18, 19, 20, 21


def _mm(a, b, dims=NN):
    return jax.lax.dot_general(a, b, dims, precision=jax.lax.Precision.DEFAULT, preferred_element_type=f32)


def _al(x, n):
    return x if isinstance(x, int) else pl.multiple_of(x, n)


def _kernel(q_hbm, k_hbm, v_hbm, shk_hbm, ssm_hbm, dv_hbm, wr_hbm, wg_hbm, wu_hbm, wd_hbm,
            c_hbm, wm_hbm, out_hbm,
            qb, kb, vb, sb, wmb, wgb, wub, wdb, shk, dv, wr, cb, cst,
            kf, kvp, sp, ub0, ub1, kp0, kp1, ypk, ypk4, y1b, y2b, st1, x1b, st2, ob, par, rb, pb, sems):
    ubs, kps = (ub0, ub1), (kp0, kp1)

    def cp(src, dst, s):
        return pltpu.make_async_copy(src, dst, sems.at[s])

    def kv_chunk(slab, it):
        c0, w = ((0, 256), (256, 384))[slab]
        rows = pl.ds(_al(it * RC, RC), RC)
        sem = S_KV + slab * NQ + it
        return [cp(k_hbm.at[0, rows, pl.ds(c0, w)], kb.at[rows, pl.ds(c0, w)], sem),
                cp(v_hbm.at[0, rows, pl.ds(c0, w)], vb.at[rows, pl.ds(c0, w)], sem)]

    def wait_kv(slab, it):
        for c in kv_chunk(slab, it):
            c.wait()

    def ssm_cp(g):
        rows = pl.ds(_al(g * 128, 128), 128)
        return cp(ssm_hbm.at[rows, :], sb.at[rows, :], S_SSM + g)

    small = [cp(shk_hbm, shk, S_SMALL), cp(dv_hbm, dv, S_SMALL), cp(wr_hbm, wr, S_SMALL), cp(c_hbm, cb, S_SMALL)]
    qc = cp(q_hbm.at[0], qb, S_Q)
    wmc = cp(wm_hbm, wmb, S_WM)
    wgc = cp(wg_hbm, wgb, S_WG)
    wuc = cp(wu_hbm, wub, S_WU)
    wdc = cp(wd_hbm, wdb, S_WD)
    order = [ssm_cp(0)] + small
    for it in range(NQ):
        order += kv_chunk(0, it)
    order += [ssm_cp(1), ssm_cp(2)]
    for it in range(NQ):
        order += kv_chunk(1, it)
    order += [ssm_cp(3), ssm_cp(4), qc, wmc, wgc, wuc, wdc]
    for c in order:
        c.start()

    ri = jax.lax.broadcasted_iota(i32, (BL, BL), 0)
    ci = jax.lax.broadcasted_iota(i32, (BL, BL), 1)

    def cos_sin(m, n):
        ang = (((4 * m + 1) * n) & (4 * BL - 1)).astype(f32) * (np.pi / (2 * BL))
        return jnp.cos(ang), jnp.sin(ang)

    def put(k, val):
        cst[64 * k:64 * (k + 1), :] = pltpu.bitcast(val.astype(bf16), u32)

    co, si = cos_sin(ri, ci)
    for k, val in enumerate((co, si - co, si + co, si + co, co, -si)):
        put(k, val)
    ct, st = cos_sin(ci, ri)
    put(6, ct * (1.0 / BL))
    put(7, st * (1.0 / BL))

    def cmat(k0, k1):
        return pltpu.bitcast(cst[64 * k0:64 * k1, :], bf16)

    for c in small:
        c.wait()
    shw = shk[...].astype(f32)
    for j in range(4):
        par[P_SH + 8 * j:P_SH + 8 * j + 8, :] = jnp.broadcast_to(shw[j:j + 1, :], (8, D))
    par[P_D:P_D + 8, :] = jnp.broadcast_to(dv[...].astype(f32).reshape(1, D), (8, D))
    for g in range(NG):
        kf[g, 0:8, :] = jnp.zeros((8, 128), f32)

    def prep_kv(g, it, s, bs):
        lanes = pl.ds(_al(g * 128, 128), 128)
        for b in bs:
            r0 = _al(it * RC + b * BL, BL)
            kblk = kb[pl.ds(r0, BL), lanes].astype(f32)
            kf[g, pl.ds(8 + r0, BL), :] = kblk
            acc = kblk.reshape(BL // 8, 8, 128) * par[P_SH:P_SH + 8, lanes][None]
            for j in range(1, 4):
                acc = acc + (kf[g, pl.ds(8 + r0 - j, BL), :].reshape(BL // 8, 8, 128)
                             * par[P_SH + 8 * j:P_SH + 8 * j + 8, lanes][None])
            kvp[s, :, b * 128:(b + 1) * 128] = acc.reshape(BL, 128) * vb[pl.ds(r0, BL), lanes].astype(f32)

    def prep_s(g, it, s, bs):
        rows = pl.ds(_al(g * 128, 128), 128)
        for b in bs:
            cols = pl.ds(_al(it * RC + b * BL, BL), BL)
            sp[s, b * 64:(b + 1) * 64, :] = pltpu.bitcast(sb[rows, cols], u32)

    def trans_u(slot, it, s):
        ubs[slot][it] = _mm(cmat(0, 3), kvp[s])

    def trans_k(slot, it, s):
        kps[slot][it] = _mm(cmat(3, 6), pltpu.bitcast(sp[s], bf16), NT)

    def conv(slot, g, rg, dst, lanes):
        r = _al(rg * 8, 8)
        dvec = par[P_D:P_D + 8, pl.ds(_al(g * 128, 128), 128)]

        def load(buf, comp, n):
            nq = -(-n // QB)
            v = buf[0:nq, pl.ds(comp * BL + r, 8), :]
            return [v[j // QB, :, (j % QB) * 128:(j % QB + 1) * 128] for j in range(n)]

        def prod(comp, init, a0, a1):
            u = load(ubs[slot], comp, a1)
            kk = load(kps[slot], comp, a1)
            if comp < 2:
                kk[0] = kk[0] + dvec
            res = {}
            for a in range(a0, a1):
                acc = u[a] * kk[0]
                if init is not None:
                    acc = acc + init[a]
                for j in range(1, a + 1):
                    acc = acc + u[a - j] * kk[j]
                res[a] = acc
            return res

        zre, zim = {}, {}
        a0 = 0
        for a1 in SPLIT:
            s1 = prod(0, None, a0, a1)
            zre.update(prod(2, s1, a0, a1))
            zim.update(prod(1, s1, a0, a1))
            yre = [zre[a] if a == 0 else zre[a] + zim[a - 1] for a in range(a0, a1)]
            yim = [zim[a] if a == 0 else zim[a] - zre[a - 1] for a in range(a0, a1)]
            dst[a0:a1, pl.ds(r, 8), lanes] = jnp.stack(yre)
            dst[a0:a1, pl.ds(BL + r, 8), lanes] = jnp.stack(yim)
            a0 = a1

    def inv03(a):
        rows = pl.ds(_al(a * BL, BL), BL)
        y1b[rows, 0:512] = _mm(cmat(6, 7), ypk[a, 0:BL, :])
        y2b[rows, 0:512] = _mm(cmat(7, 8), ypk[a, BL:2 * BL, :])

    def inv4(a0):
        o1 = _mm(cmat(6, 7), jnp.concatenate([ypk4[a0 + b, 0:BL, :] for b in range(L2N)], axis=1))
        o2 = _mm(cmat(7, 8), jnp.concatenate([ypk4[a0 + b, BL:2 * BL, :] for b in range(L2N)], axis=1))
        for b in range(L2N):
            rows = pl.ds(_al((a0 + b) * BL, BL), BL)
            y1b[rows, 512:640] = o1[:, b * 128:(b + 1) * 128]
            y2b[rows, 512:640] = o2[:, b * 128:(b + 1) * 128]

    def stats(x, dst, rows):
        m = jnp.sum(x, axis=-1, keepdims=True) * (1.0 / D)
        ex2 = jnp.sum(x * x, axis=-1, keepdims=True) * (1.0 / D)
        rs = jax.lax.rsqrt(jnp.maximum(ex2 - m * m, 0.0) + EPS)
        dst[0, rows, :] = jnp.broadcast_to(m, (BL, 128))
        dst[1, rows, :] = jnp.broadcast_to(rs, (BL, 128))

    allb = range(QB)
    ssm_cp(0).wait()
    for it in range(NQ):
        prep_s(0, it, it, allb)
    trans_k(0, 0, 0)
    for it in range(NQ):
        wait_kv(0, it)
        prep_kv(0, it, it, allb)
        if it + 1 < NQ:
            trans_k(0, it + 1, it + 1)
        if it > 0:
            trans_u(0, it - 1, it - 1)
    ssm_cp(1).wait()
    prep_kv(1, 0, NQ, allb)
    prep_s(1, 0, NQ, allb)
    trans_u(0, NQ - 1, NQ - 1)

    def pair(p, carry):
        for par_ in range(2):
            g = 2 * p + par_

            def step(it, c, par_=par_, g=g):
                last = it == NQ - 1
                if par_ == 0:
                    @pl.when(last)
                    def _():
                        ssm_cp(g + 2).wait()

                    @pl.when(jnp.logical_and(last, p == 0))
                    def _():
                        wait_kv(1, 0)
                else:
                    @pl.when(jnp.logical_and(jnp.logical_not(last), p == 0))
                    def _():
                        wait_kv(1, jnp.minimum(it + 1, NQ - 1))

                    @pl.when(jnp.logical_and(last, p == 0))
                    def _():
                        ssm_cp(3).wait()
                s = (g + 1) * NQ + it
                gn = jnp.minimum(g + 1 + (it + 1) // NQ, NG - 1)
                itn = (it + 1) % NQ
                lanes = pl.ds(_al(g * 128, 128), 128)
                for bs in ((0,), (1,), (2,)):
                    prep_kv(gn, itn, s + 1, bs)
                    prep_s(gn, itn, s + 1, bs)
                for b in range(QB):
                    conv(par_, g, it * QB + b, ypk, lanes)
                trans_u(1 - par_, it, s)
                trans_k(1 - par_, it, s)
                prep_kv(gn, itn, s + 1, (3,))
                prep_s(gn, itn, s + 1, (3,))
                return c
            jax.lax.fori_loop(0, NQ, step, 0)
        return carry
    jax.lax.fori_loop(0, 2, pair, 0)

    qc.wait()

    def last_group(it, c):
        for b in range(QB):
            rows = pl.ds(_al((it * QB + b) * BL, BL), BL)
            stats(qb[rows, :].astype(f32), st1, rows)
        for b in range(QB):
            conv(0, NG - 1, it * QB + b, ypk4, slice(None))
        for b in range(QB):
            inv03(it * QB + b)
        return c
    jax.lax.fori_loop(0, NQ, last_group, 0)

    wmc.wait()
    inv4(0)
    cv = cb[...].astype(f32)
    sc = (cv * jax.nn.sigmoid(cv)).astype(bf16)
    mod = _mm(jnp.broadcast_to(sc, (8, D)), wmb[...])
    sa, ca, ga, sb_, cb_, gb = [mod[:, j * D:(j + 1) * D] for j in range(6)]
    par[P_A1:P_A1 + 8, :] = ga * (1.0 + ca)
    par[P_B1:P_B1 + 8, :] = ga * sa
    par[P_A2:P_A2 + 8, :] = gb * (1.0 + cb_)
    par[P_B2:P_B2 + 8, :] = gb * sb_
    par[P_C2:P_C2 + 8, :] = 1.0 + cb_
    par[P_S2:P_S2 + 8, :] = sb_
    par[P_G2:P_G2 + 8, :] = gb
    wrv = jnp.broadcast_to(wr[...].astype(f32).reshape(1, D), (8, D))
    wp = (1.0 + cb_) * wrv
    wp_hi = wp.astype(bf16).astype(f32)
    row8 = jax.lax.broadcasted_iota(i32, (8, D), 0)
    par[P_WR:P_WR + 8, :] = jnp.where(row8 == 0, wp_hi, jnp.where(row8 == 1, wp - wp_hi, 0.0))
    rconst = jnp.sum(sb_[0:1, :] * wrv[0:1, :], axis=-1, keepdims=True)

    def tile5(t):
        return jnp.concatenate([t] * NG, axis=1)

    def affine(n, pa, pb_):
        t = n.reshape(BL // 8, 8, D) * par[pa:pa + 8, :][None] + par[pb_:pb_ + 8, :][None]
        return t.reshape(BL, D)

    def stage_a(i):
        rows = pl.ds(_al(i * BL, BL), BL)
        y = y1b[rows, :] + y2b[rows, :]
        x = qb[rows, :].astype(f32)
        n1 = (x - tile5(st1[0, rows, :])) * tile5(st1[1, rows, :])
        x1 = x + affine(n1, P_A1, P_B1) * y
        x1b[rows, :] = x1
        stats(x1, st2, rows)

    def stage_b(i):
        rows = pl.ds(_al(i * BL, BL), BL)
        x1 = x1b[rows, :]
        n2 = (x1 - tile5(st2[0, rows, :])) * tile5(st2[1, rows, :])
        ob[rows, :] = (x1 + affine(n2, P_A2, P_B2)).astype(bf16)
        rr = _mm(par[P_WR:P_WR + 8, :], n2, NT)
        rb[pl.ds(i, 1), :] = rr[0:1, :] + rr[1:2, :]

    n2it = NB // L2N

    def l2_body(i, do_m, do_a, do_b):
        if do_b:
            for b in range(L2N):
                stage_b((i - 1) * L2N + b)
        if do_a:
            for b in range(L2N):
                stage_a(i * L2N + b)
        if do_m:
            inv4((i + 1) * L2N)

    def out_cp(a):
        rows = pl.ds(_al(a * BL, BL), BL)
        return cp(ob.at[rows, :], out_hbm.at[0, rows, :], S_OE if isinstance(a, int) and a < NE else S_OL)

    l2_body(0, True, True, False)

    def l2(i, c):
        l2_body(i, True, True, True)
        return c
    jax.lax.fori_loop(1, n2it - 1, l2, 0)
    l2_body(n2it - 1, False, True, True)
    for a in range(NE):
        out_cp(a).start()
    l2_body(n2it, False, False, True)

    r = rb[...] + rconst
    posf = (jax.lax.broadcasted_iota(i32, (NB, BL), 0) * BL
            + jax.lax.broadcasted_iota(i32, (NB, BL), 1)).astype(f32)

    def allmax(t):
        return jnp.max(jnp.max(t, axis=1, keepdims=True), axis=0, keepdims=True)

    def allmin(t):
        return jnp.min(jnp.min(t, axis=1, keepdims=True), axis=0, keepdims=True)

    m1 = allmax(r)
    p1 = allmin(jnp.where(r == m1, posf, float(S)))
    r2 = jnp.where(posf == p1, -jnp.inf, r)
    m2 = allmax(r2)
    p2 = allmin(jnp.where(jnp.logical_and(r2 == m2, posf != p1), posf, float(S)))
    i1 = jnp.clip(p1[0, 0].astype(i32), 0, S - 1)
    i2 = jnp.clip(p2[0, 0].astype(i32), 0, S - 1)
    a1 = i1 // BL
    a2 = i2 // BL
    for a in range(NE, NB):
        @pl.when(jnp.logical_and(a1 != a, a2 != a))
        def _(a=a):
            out_cp(a).start()

    def sel_row(idx):
        x1 = x1b[pl.ds(idx, 1), :]
        n2 = (x1 - tile5(st2[0, pl.ds(idx, 1), :])) * tile5(st2[1, pl.ds(idx, 1), :])
        return x1, n2 * par[P_C2:P_C2 + 1, :] + par[P_S2:P_S2 + 1, :]
    xa, ha = sel_row(i1)
    xb, hb = sel_row(i2)
    hs = jnp.where(row8 == 0, ha, jnp.where(row8 == 1, hb, 0.0)).astype(bf16)
    wgc.wait()
    gate = _mm(hs, wgb[...], NT)
    wuc.wait()
    up = _mm(hs, wub[...], NT)
    act = (gate * jax.nn.sigmoid(gate) * up).astype(bf16)
    wdc.wait()
    ymoe = _mm(act, wdb[...])
    gbv = par[P_G2:P_G2 + 1, :]
    oa = xa + gbv * (ha + ymoe[0:1, :] * jax.nn.sigmoid(m1))
    obb = xb + gbv * (hb + ymoe[1:2, :] * jax.nn.sigmoid(m2))
    row16 = jax.lax.broadcasted_iota(i32, (16, D), 0)
    b1 = pl.multiple_of((i1 // 16) * 16, 16)
    b2 = pl.multiple_of((i2 // 16) * 16, 16)
    for n, base in enumerate((b1, b2)):
        blk = ob[pl.ds(base, 16), :].astype(f32)
        blk = jnp.where(row16 == i1 - base, oa, jnp.where(row16 == i2 - base, obb, blk))
        pb[n] = blk.astype(bf16)
    for a in range(NE):
        out_cp(a).wait()

    def tile_cp(n, base):
        return cp(pb.at[n], out_hbm.at[0, pl.ds(base, 16), :], S_OE)

    e1 = a1 < NE
    e2 = jnp.logical_and(a2 < NE, b2 != b1)

    @pl.when(e1)
    def _():
        tile_cp(0, b1).start()

    @pl.when(e2)
    def _():
        tile_cp(1, b2).start()

    @pl.when(a1 >= NE)
    def _():
        ob[pl.ds(b1, 16), :] = pb[0]

    @pl.when(a2 >= NE)
    def _():
        ob[pl.ds(b2, 16), :] = pb[1]

    @pl.when(a1 >= NE)
    def _():
        out_cp(a1).start()

    @pl.when(jnp.logical_and(a2 >= NE, a2 != a1))
    def _():
        out_cp(a2).start()

    for a in range(NE, NB):
        out_cp(a).wait()

    @pl.when(e1)
    def _():
        tile_cp(0, b1).wait()

    @pl.when(e2)
    def _():
        tile_cp(1, b2).wait()


@jax.jit
def pallas_adaLN_cond__ssm_conv_h3__moe_arch_mod__prompt_kernel(
    A_q, A_k, A_v, A_shift_k, A_ssm_k, A_ssm_D, B_x, B_w_r, B_w_gate, B_w_up, B_w_down, c, w_mod,
):
    del B_x
    anyspec = pl.BlockSpec(memory_space=pl.ANY)
    V = pltpu.VMEM
    scratch = [
        V((S, D), bf16), V((S, D), bf16), V((S, D), bf16), V((D, S), bf16),
        V((D, 6 * D), bf16), V((FF, D), bf16), V((FF, D), bf16), V((FF, D), bf16),
        V((4, D), bf16), V((D,), bf16), V((D,), bf16), V((1, D), bf16),
        V((512, 128), u32),
        V((NG, S + 8, 128), f32),
        V((NG * NQ + 1, BL, QB * 128), f32),
        V((NG * NQ + 1, QB * 64, 128), u32),
        V((NQ, 3 * BL, QB * 128), f32), V((NQ, 3 * BL, QB * 128), f32),
        V((NQ, 3 * BL, QB * 128), f32), V((NQ, 3 * BL, QB * 128), f32),
        V((NB, 2 * BL, 512), f32), V((NB, 2 * BL, 128), f32),
        V((S, D), f32), V((S, D), f32),
        V((2, S, 128), f32),
        V((S, D), f32),
        V((2, S, 128), f32),
        V((S, D), bf16),
        V((P_END, D), f32),
        V((NB, BL), f32),
        V((2, 16, D), bf16),
        pltpu.SemaphoreType.DMA((S_END,)),
    ]
    return pl.pallas_call(
        _kernel,
        out_shape=jax.ShapeDtypeStruct((1, S, D), bf16),
        in_specs=[anyspec] * 12,
        out_specs=anyspec,
        scratch_shapes=scratch,
        compiler_params=pltpu.CompilerParams(vmem_limit_bytes=100 * 1024 * 1024,
                                             disable_bounds_checks=True, disable_semaphore_checks=True),
        name="ssm_moe",
    )(A_q, A_k, A_v, A_shift_k.T, A_ssm_k, A_ssm_D, B_w_r, B_w_gate.T, B_w_up.T, B_w_down, c, w_mod)
```

```python
import numpy as np
import jax
import jax.numpy as jnp
import jax.experimental.pallas as pl
import jax.experimental.pallas.tpu as pltpu

S, D, FF = 2048, 640, 1728
BL = 128
NB = S // BL
NG = D // 128
QB = 4
NQ = NB // QB
RC = QB * BL
L2N = 2
NE = NB - 3 * L2N
SPLIT = (10, 16)
EPS = 1e-5
WDX = 256
f32, bf16, u32, i32 = jnp.float32, jnp.bfloat16, jnp.uint32, jnp.int32
NT = (((1,), (1,)), ((), ()))
NN = (((1,), (0,)), ((), ()))

P_SH, P_D, P_A1, P_B1, P_A2, P_B2, P_C2, P_S2, P_G2, P_WR, P_END = 0, 32, 40, 48, 56, 64, 72, 80, 88, 96, 104
S_SMALL, S_KV, S_SSM, S_Q, S_WM, S_WG, S_WU, S_WD, S_OE, S_WD2, S_END = 0, 1, 9, 14, 15, 16, 17, 18, 19, 20, 21


def _mm(a, b, dims=NN):
    return jax.lax.dot_general(a, b, dims, precision=jax.lax.Precision.DEFAULT, preferred_element_type=f32)


def _al(x, n):
    return x if isinstance(x, int) else pl.multiple_of(x, n)


def _kernel(q_hbm, k_hbm, v_hbm, shk_hbm, ssm_hbm, dv_hbm, wr_hbm, wg_hbm, wu_hbm, wd_hbm,
            c_hbm, wm_hbm, out_hbm,
            qb, kb, vb, sb, wmb, wgb, wub, wdb, shk, dv, wr, cb, cst,
            kf, kvp, sp, ub0, ub1, kp0, kp1, ypk, ypk4, y1b, y2b, st1, x1b, st2, ob, par, rb, sems):
    ubs, kps = (ub0, ub1), (kp0, kp1)

    def cp(src, dst, s):
        return pltpu.make_async_copy(src, dst, sems.at[s])

    def kv_chunk(slab, it):
        c0, w = ((0, 256), (256, 384))[slab]
        rows = pl.ds(_al(it * RC, RC), RC)
        sem = S_KV + slab * NQ + it
        return [cp(k_hbm.at[0, rows, pl.ds(c0, w)], kb.at[rows, pl.ds(c0, w)], sem),
                cp(v_hbm.at[0, rows, pl.ds(c0, w)], vb.at[rows, pl.ds(c0, w)], sem)]

    def wait_kv(slab, it):
        for c in kv_chunk(slab, it):
            c.wait()

    def ssm_cp(g):
        rows = pl.ds(_al(g * 128, 128), 128)
        return cp(ssm_hbm.at[rows, :], sb.at[rows, :], S_SSM + g)

    small = [cp(shk_hbm, shk, S_SMALL), cp(dv_hbm, dv, S_SMALL), cp(wr_hbm, wr, S_SMALL), cp(c_hbm, cb, S_SMALL)]
    qc = cp(q_hbm.at[0], qb, S_Q)
    wmc = cp(wm_hbm, wmb, S_WM)
    wgc = cp(wg_hbm, wgb, S_WG)
    wuc = cp(wu_hbm, wub, S_WU)
    wdc = cp(wd_hbm.at[pl.ds(0, FF - WDX), :], wdb.at[pl.ds(0, FF - WDX), :], S_WD)
    wdc2 = cp(wd_hbm.at[pl.ds(FF - WDX, WDX), :], wdb.at[pl.ds(FF - WDX, WDX), :], S_WD2)
    order = [ssm_cp(0)] + small
    for it in range(NQ):
        order += kv_chunk(0, it)
    order += [ssm_cp(1), ssm_cp(2)]
    for it in range(NQ):
        order += kv_chunk(1, it)
    order += [ssm_cp(3), ssm_cp(4), qc, wmc, wgc, wuc, wdc, wdc2]
    for c in order:
        c.start()

    ri = jax.lax.broadcasted_iota(i32, (BL, BL), 0)
    ci = jax.lax.broadcasted_iota(i32, (BL, BL), 1)

    def cos_sin(m, n):
        ang = (((4 * m + 1) * n) & (4 * BL - 1)).astype(f32) * (np.pi / (2 * BL))
        return jnp.cos(ang), jnp.sin(ang)

    def put(k, val):
        cst[64 * k:64 * (k + 1), :] = pltpu.bitcast(val.astype(bf16), u32)

    co, si = cos_sin(ri, ci)
    for k, val in enumerate((co, si - co, si + co, si + co, co, -si)):
        put(k, val)
    ct, st = cos_sin(ci, ri)
    put(6, ct * (1.0 / BL))
    put(7, st * (1.0 / BL))

    def cmat(k0, k1):
        return pltpu.bitcast(cst[64 * k0:64 * k1, :], bf16)

    for c in small:
        c.wait()
    shw = shk[...].astype(f32)
    for j in range(4):
        par[P_SH + 8 * j:P_SH + 8 * j + 8, :] = jnp.broadcast_to(shw[j:j + 1, :], (8, D))
    par[P_D:P_D + 8, :] = jnp.broadcast_to(dv[...].astype(f32).reshape(1, D), (8, D))
    for g in range(NG):
        kf[g, 0:8, :] = jnp.zeros((8, 128), f32)
    rb[...] = jnp.zeros((NB, BL), f32)

    def prep_kv(g, it, s, bs):
        lanes = pl.ds(_al(g * 128, 128), 128)
        for b in bs:
            r0 = _al(it * RC + b * BL, BL)
            kblk = kb[pl.ds(r0, BL), lanes].astype(f32)
            kf[g, pl.ds(8 + r0, BL), :] = kblk
            acc = kblk.reshape(BL // 8, 8, 128) * par[P_SH:P_SH + 8, lanes][None]
            for j in range(1, 4):
                acc = acc + (kf[g, pl.ds(8 + r0 - j, BL), :].reshape(BL // 8, 8, 128)
                             * par[P_SH + 8 * j:P_SH + 8 * j + 8, lanes][None])
            kvp[s, :, b * 128:(b + 1) * 128] = acc.reshape(BL, 128) * vb[pl.ds(r0, BL), lanes].astype(f32)

    def prep_s(g, it, s, bs):
        rows = pl.ds(_al(g * 128, 128), 128)
        for b in bs:
            cols = pl.ds(_al(it * RC + b * BL, BL), BL)
            sp[s, b * 64:(b + 1) * 64, :] = pltpu.bitcast(sb[rows, cols], u32)

    def trans_u(slot, it, s):
        ubs[slot][it] = _mm(cmat(0, 3), kvp[s])

    def trans_k(slot, it, s):
        kps[slot][it] = _mm(cmat(3, 6), pltpu.bitcast(sp[s], bf16), NT)

    def conv(slot, rg, dst, lanes):
        r = _al(rg * 8, 8)

        def load(buf, comp, n):
            nq = -(-n // QB)
            v = buf[0:nq, pl.ds(comp * BL + r, 8), :]
            return [v[j // QB, :, (j % QB) * 128:(j % QB + 1) * 128] for j in range(n)]

        def prod(comp, init, a0, a1):
            u = load(ubs[slot], comp, a1)
            kk = load(kps[slot], comp, a1)
            res = {}
            for a in range(a0, a1):
                acc = u[a] * kk[0]
                if init is not None:
                    acc = acc + init[a]
                for j in range(1, a + 1):
                    acc = acc + u[a - j] * kk[j]
                res[a] = acc
            return res

        zre, zim = {}, {}
        a0 = 0
        for a1 in SPLIT:
            s1 = prod(0, None, a0, a1)
            zre.update(prod(2, s1, a0, a1))
            zim.update(prod(1, s1, a0, a1))
            yre = [zre[a] if a == 0 else zre[a] + zim[a - 1] for a in range(a0, a1)]
            yim = [zim[a] if a == 0 else zim[a] - zre[a - 1] for a in range(a0, a1)]
            dst[a0:a1, pl.ds(r, 8), lanes] = jnp.stack(yre)
            dst[a0:a1, pl.ds(BL + r, 8), lanes] = jnp.stack(yim)
            a0 = a1

    def inv03(a):
        rows = pl.ds(_al(a * BL, BL), BL)
        y1b[rows, 0:512] = _mm(cmat(6, 7), ypk[a, 0:BL, :])
        y2b[rows, 0:512] = _mm(cmat(7, 8), ypk[a, BL:2 * BL, :])

    def inv4(a0):
        o1 = _mm(cmat(6, 7), jnp.concatenate([ypk4[a0 + b, 0:BL, :] for b in range(L2N)], axis=1))
        o2 = _mm(cmat(7, 8), jnp.concatenate([ypk4[a0 + b, BL:2 * BL, :] for b in range(L2N)], axis=1))
        for b in range(L2N):
            rows = pl.ds(_al((a0 + b) * BL, BL), BL)
            y1b[rows, 512:640] = o1[:, b * 128:(b + 1) * 128]
            y2b[rows, 512:640] = o2[:, b * 128:(b + 1) * 128]

    def stats(x, dst, rows):
        m = jnp.sum(x, axis=-1, keepdims=True) * (1.0 / D)
        ex2 = jnp.sum(x * x, axis=-1, keepdims=True) * (1.0 / D)
        rs = jnp.exp(-0.5 * jnp.log(jnp.maximum(ex2 - m * m, 0.0) + EPS))
        dst[0, rows, :] = jnp.broadcast_to(m, (BL, 128))
        dst[1, rows, :] = jnp.broadcast_to(rs, (BL, 128))

    allb = range(QB)
    ssm_cp(0).wait()
    for it in range(NQ):
        prep_s(0, it, it, allb)
    trans_k(0, 0, 0)
    for it in range(NQ):
        wait_kv(0, it)
        prep_kv(0, it, it, allb)
        if it + 1 < NQ:
            trans_k(0, it + 1, it + 1)
        if it > 0:
            trans_u(0, it - 1, it - 1)
    ssm_cp(1).wait()
    prep_kv(1, 0, NQ, allb)
    prep_s(1, 0, NQ, allb)
    trans_u(0, NQ - 1, NQ - 1)

    def pair(p, carry):
        for par_ in range(2):
            g = 2 * p + par_

            def step(it, c, par_=par_, g=g):
                last = it == NQ - 1
                if par_ == 0:
                    @pl.when(last)
                    def _():
                        ssm_cp(g + 2).wait()

                    @pl.when(jnp.logical_and(last, p == 0))
                    def _():
                        wait_kv(1, 0)
                else:
                    @pl.when(jnp.logical_and(jnp.logical_not(last), p == 0))
                    def _():
                        wait_kv(1, jnp.minimum(it + 1, NQ - 1))

                    @pl.when(jnp.logical_and(last, p == 0))
                    def _():
                        ssm_cp(3).wait()
                s = (g + 1) * NQ + it
                gn = jnp.minimum(g + 1 + (it + 1) // NQ, NG - 1)
                itn = (it + 1) % NQ
                lanes = pl.ds(_al(g * 128, 128), 128)
                for bs in ((0,), (1,), (2,)):
                    prep_kv(gn, itn, s + 1, bs)
                    prep_s(gn, itn, s + 1, bs)
                for b in range(QB):
                    conv(par_, it * QB + b, ypk, lanes)
                trans_u(1 - par_, it, s)
                trans_k(1 - par_, it, s)
                prep_kv(gn, itn, s + 1, (3,))
                prep_s(gn, itn, s + 1, (3,))
                return c
            jax.lax.fori_loop(0, NQ, step, 0)
        return carry
    jax.lax.fori_loop(0, 2, pair, 0)

    qc.wait()

    def last_group(it, c):
        for b in range(QB):
            rows = pl.ds(_al((it * QB + b) * BL, BL), BL)
            stats(qb[rows, :].astype(f32), st1, rows)
        for b in range(QB):
            conv(0, it * QB + b, ypk4, slice(None))
        for b in range(QB):
            inv03(it * QB + b)
        return c
    jax.lax.fori_loop(0, NQ, last_group, 0)

    wmc.wait()
    inv4(0)
    cv = cb[...].astype(f32)
    sc = (cv * jax.nn.sigmoid(cv)).astype(bf16)
    mod = _mm(jnp.broadcast_to(sc, (8, D)), wmb[...])
    sa, ca, ga, sb_, cb_, gb = [mod[:, j * D:(j + 1) * D] for j in range(6)]
    par[P_A1:P_A1 + 8, :] = ga * (1.0 + ca)
    par[P_B1:P_B1 + 8, :] = ga * sa
    par[P_A2:P_A2 + 8, :] = gb * (1.0 + cb_)
    par[P_B2:P_B2 + 8, :] = gb * sb_
    par[P_C2:P_C2 + 8, :] = 1.0 + cb_
    par[P_S2:P_S2 + 8, :] = sb_
    par[P_G2:P_G2 + 8, :] = gb
    wrv = jnp.broadcast_to(wr[...].astype(f32).reshape(1, D), (8, D))
    wp = (1.0 + cb_) * wrv
    wp_hi = wp.astype(bf16).astype(f32)
    row8 = jax.lax.broadcasted_iota(i32, (8, D), 0)
    par[P_WR:P_WR + 8, :] = jnp.where(row8 == 0, wp_hi, jnp.where(row8 == 1, wp - wp_hi, 0.0))
    rconst = jnp.sum(sb_[0:1, :] * wrv[0:1, :], axis=-1, keepdims=True)

    def tile5(t):
        return jnp.concatenate([t] * NG, axis=1)

    def affine(n, pa, pb_):
        t = n.reshape(BL // 8, 8, D) * par[pa:pa + 8, :][None] + par[pb_:pb_ + 8, :][None]
        return t.reshape(BL, D)

    def stage_a(i):
        rows = pl.ds(_al(i * BL, BL), BL)
        cols = pl.ds(_al((i % QB) * 128, 128), 128)
        kv = jnp.concatenate([kvp[g * NQ + i // QB, :, cols] for g in range(NG)], axis=1)
        y = y1b[rows, :] + y2b[rows, :] + (kv.reshape(BL // 8, 8, D) * par[P_D:P_D + 8, :][None]).reshape(BL, D)
        x = qb[rows, :].astype(f32)
        n1 = (x - tile5(st1[0, rows, :])) * tile5(st1[1, rows, :])
        x1 = x + affine(n1, P_A1, P_B1) * y
        x1b[rows, :] = x1
        stats(x1, st2, rows)

    def stage_b(i):
        rows = pl.ds(_al(i * BL, BL), BL)
        x1 = x1b[rows, :]
        n2 = (x1 - tile5(st2[0, rows, :])) * tile5(st2[1, rows, :])
        ob[rows, :] = (x1 + affine(n2, P_A2, P_B2)).astype(bf16)
        rr = _mm(par[P_WR:P_WR + 8, :], n2, NT)
        rb[pl.ds(i, 1), :] = rr[0:1, :] + rr[1:2, :]

    n2it = NB // L2N

    def l2_body(i, do_m, do_a, do_b):
        if do_b:
            for b in range(L2N):
                stage_b((i - 1) * L2N + b)
        if do_a:
            for b in range(L2N):
                stage_a(i * L2N + b)
        if do_m:
            inv4((i + 1) * L2N)

    def out_cp(a):
        rows = pl.ds(_al(a * BL, BL), BL)
        return cp(ob.at[rows, :], out_hbm.at[0, rows, :], S_OE)

    l2_body(0, True, True, False)

    def l2(i, c):
        l2_body(i, True, True, True)
        return c
    jax.lax.fori_loop(1, n2it - 2, l2, 0)
    low = S - 1
    big = float(np.finfo(np.float32).max)

    def allmax(t):
        return jnp.max(jnp.max(t, axis=0, keepdims=True), axis=1, keepdims=True)

    def decode(k):
        kb_ = pltpu.bitcast(jnp.broadcast_to(k, (8, 128)), i32)[0:1, 0:1]
        return jnp.where(kb_ < 0, kb_ & low, low - (kb_ & low))[0, 0]

    def top2(nrows):
        r = rb[...] + rconst
        blk = jax.lax.broadcasted_iota(i32, (NB, BL), 0)
        pos = blk * BL + jax.lax.broadcasted_iota(i32, (NB, BL), 1)
        if nrows < NB:
            r = jnp.where(blk < nrows, r, -big)
        bits = pltpu.bitcast(jnp.where(r == r, jnp.clip(r, -big, big), -big), i32)
        key = pltpu.bitcast((bits & ~low) | jnp.where(bits < 0, pos, low - pos), f32)
        k1 = allmax(key)
        k2 = allmax(jnp.where(key == k1, -jnp.inf, key))
        return r, key, k1, k2

    _, _, pk1, pk2 = top2(NE)
    l2_body(n2it - 2, True, True, True)
    pa1 = decode(pk1) // BL
    pa2 = decode(pk2) // BL

    def early(a):
        return jnp.logical_and(a < NE, jnp.logical_and(a != pa1, a != pa2))

    wdc.wait()
    for a in range(NE):
        @pl.when(early(a))
        def _(a=a):
            out_cp(a).start()
    l2_body(n2it - 1, False, True, True)
    l2_body(n2it, False, False, True)

    r, key, k1, k2 = top2(NB)
    m1 = allmax(jnp.where(key == k1, r, -jnp.inf))
    m2 = allmax(jnp.where(key == k2, r, -jnp.inf))
    i1 = decode(k1)
    i2 = decode(k2)
    a1 = i1 // BL
    a2 = i2 // BL
    for a in range(NB):
        @pl.when(jnp.logical_and(jnp.logical_not(early(a)), jnp.logical_and(a1 != a, a2 != a)))
        def _(a=a):
            out_cp(a).start()

    wgc.wait()
    wuc.wait()

    def sel_row(idx):
        x1 = x1b[pl.ds(idx, 1), :]
        n2 = (x1 - tile5(st2[0, pl.ds(idx, 1), :])) * tile5(st2[1, pl.ds(idx, 1), :])
        return x1, n2 * par[P_C2:P_C2 + 1, :] + par[P_S2:P_S2 + 1, :]
    xa, ha = sel_row(i1)
    xb, hb = sel_row(i2)
    hs = jnp.where(row8 == 0, ha, jnp.where(row8 == 1, hb, 0.0)).astype(bf16)
    gate = _mm(hs, wgb[...], NT)
    up = _mm(hs, wub[...], NT)
    act = (gate * jax.nn.sigmoid(gate) * up).astype(bf16)
    wdc2.wait()
    ymoe = _mm(act, wdb[...])
    gbv = par[P_G2:P_G2 + 1, :]
    oa = xa + gbv * (ha + ymoe[0:1, :] * jax.nn.sigmoid(m1))
    obb = xb + gbv * (hb + ymoe[1:2, :] * jax.nn.sigmoid(m2))
    row16 = jax.lax.broadcasted_iota(i32, (16, D), 0)
    for idx, a, val in ((i1, a1, oa), (i2, a2, obb)):
        @pl.when(jnp.logical_not(early(a)))
        def _(idx=idx, val=val):
            base = pl.multiple_of((idx // 16) * 16, 16)
            blk = ob[pl.ds(base, 16), :].astype(f32)
            ob[pl.ds(base, 16), :] = jnp.where(row16 == idx - base, val, blk).astype(bf16)

    @pl.when(jnp.logical_not(early(a1)))
    def _():
        out_cp(a1).start()

    @pl.when(jnp.logical_and(jnp.logical_not(early(a2)), a2 != a1))
    def _():
        out_cp(a2).start()

    for a in range(NB):
        out_cp(a).wait()


@jax.jit
def pallas_adaLN_cond__ssm_conv_h3__moe_arch_mod__prompt_kernel(
    A_q, A_k, A_v, A_shift_k, A_ssm_k, A_ssm_D, B_x, B_w_r, B_w_gate, B_w_up, B_w_down, c, w_mod,
):
    del B_x
    anyspec = pl.BlockSpec(memory_space=pl.ANY)
    V = pltpu.VMEM
    scratch = [
        V((S, D), bf16), V((S, D), bf16), V((S, D), bf16), V((D, S), bf16),
        V((D, 6 * D), bf16), V((FF, D), bf16), V((FF, D), bf16), V((FF, D), bf16),
        V((4, D), bf16), V((D,), bf16), V((D,), bf16), V((1, D), bf16),
        V((512, 128), u32),
        V((NG, S + 8, 128), f32),
        V((NG * NQ + 1, BL, QB * 128), f32),
        V((NG * NQ + 1, QB * 64, 128), u32),
        V((NQ, 3 * BL, QB * 128), f32), V((NQ, 3 * BL, QB * 128), f32),
        V((NQ, 3 * BL, QB * 128), f32), V((NQ, 3 * BL, QB * 128), f32),
        V((NB, 2 * BL, 512), f32), V((NB, 2 * BL, 128), f32),
        V((S, D), f32), V((S, D), f32),
        V((2, S, 128), f32),
        V((S, D), f32),
        V((2, S, 128), f32),
        V((S, D), bf16),
        V((P_END, D), f32),
        V((NB, BL), f32),
        pltpu.SemaphoreType.DMA((S_END,)),
    ]
    return pl.pallas_call(
        _kernel,
        out_shape=jax.ShapeDtypeStruct((1, S, D), bf16),
        in_specs=[anyspec] * 12,
        out_specs=anyspec,
        scratch_shapes=scratch,
        compiler_params=pltpu.CompilerParams(vmem_limit_bytes=100 * 1024 * 1024,
                                             disable_bounds_checks=True, disable_semaphore_checks=True),
        name="ssm_moe",
    )(A_q, A_k, A_v, A_shift_k.T, A_ssm_k, A_ssm_D, B_w_r, B_w_gate.T, B_w_up.T, B_w_down, c, w_mod)
```
